```python
import jax
import jax.numpy as jnp

def _softmax(x, axis=-1):
    return jax.nn.softmax(x, axis=axis)
def _gelu(x):
    return jax.nn.gelu(x, approximate=True)
def _silu(x):
    return jax.nn.silu(x)
def _sigmoid(x):
    return jax.nn.sigmoid(x)
def _layernorm(x, axis=-1, eps=1e-5):
    m = jnp.mean(x, axis=axis, keepdims=True)
    v = jnp.var(x, axis=axis, keepdims=True)
    return (x - m) / jnp.sqrt(v + eps)
def _scatter_add(tgt, idx, src, axis=0):
    return tgt.at[idx].add(src)
def _segment_sum(src, seg, n):
    return jax.ops.segment_sum(src, seg, n)
class _Rng:
    def __init__(self, key):
        self._k = key
    def _next(self):
        self._k, sub = jax.random.split(self._k)
        return sub
    def normal(self, shape):
        return jax.random.normal(self._next(), shape, dtype=jnp.bfloat16)
    def randint(self, lo, hi, shape):
        return jax.random.randint(self._next(), shape, lo, hi, dtype=jnp.int32)
    def uniform(self, shape, lo=0.0, hi=1.0):
        return jax.random.uniform(self._next(), shape, jnp.bfloat16, lo, hi)
    def permutation(self, n):
        return jax.random.permutation(self._next(), n)


kernel_name = 'sequential_preLN__sliding_block_cached__moe_arch_mod__decode'

def setup_inputs():
    _rng = _Rng(jax.random.key(int.from_bytes(__import__("os").urandom(4), "little")))
    _w = (lambda a: (lambda t: t.astype(jnp.bfloat16) if jnp.issubdtype(t.dtype, jnp.floating) else t)(jnp.asarray(a)))
    def _A_setup():
        B, Sq, D = 1, 1, 640
        Hq, Hkv, Sk, Dh = 32, 32, 32768, 192
        assert Hq % Hkv == 0, (Hq, Hkv)
        return {
            "x": _w((lambda *s: _rng.normal(s) * 0.05)(B, Sq, D)),
            "k_cache": _w((lambda *s: _rng.normal(s) * 0.05)(B, Hkv, Sk, Dh)),
            "v_cache": _w((lambda *s: _rng.normal(s) * 0.05)(B, Hkv, Sk, Dh)),
            "wq": _w((lambda *s: _rng.normal(s) * 0.05)(D, Hq * Dh) * (D ** -0.5)),
            "wo": _w((lambda *s: _rng.normal(s) * 0.05)(Hq * Dh, D) * ((Hq * Dh) ** -0.5)),
        }
    _A_in = _A_setup()

    def _B_setup():
        B, S, D, F, C = 1, 1, 640, 1536, 1
        return {
            "x": _w((lambda *s: _rng.normal(s) * 0.05)(B, S, D)),
            "w_r": _w((lambda *s: _rng.normal(s) * 0.05)(D)),
            "w_gate": _w((lambda *s: _rng.normal(s) * 0.05)(D, F)),
            "w_up": _w((lambda *s: _rng.normal(s) * 0.05)(D, F)),
            "w_down": _w((lambda *s: _rng.normal(s) * 0.05)(F, D)),
        }
    _B_in = _B_setup()

    return {
        "A_x": _A_in["x"],
        "A_k_cache": _A_in["k_cache"],
        "A_v_cache": _A_in["v_cache"],
        "A_wq": _A_in["wq"],
        "A_wo": _A_in["wo"],
        "B_x": _B_in["x"],
        "B_w_r": _B_in["w_r"],
        "B_w_gate": _B_in["w_gate"],
        "B_w_up": _B_in["w_up"],
        "B_w_down": _B_in["w_down"],
    }

def reference(A_x, A_k_cache, A_v_cache, A_wq, A_wo, B_x, B_w_r, B_w_gate, B_w_up, B_w_down):
    def _A_ref(x, k_cache, v_cache, wq, wo):
        B, Sq, D = x.shape
        Hq, Dh = 32, 192
        Hkv, Sk = k_cache.shape[1], k_cache.shape[2]
        W = min(4096, max(256, Sk // 4))
        rep = Hq // Hkv
        q = (lambda x, *d: x.transpose(*d))((x @ wq).reshape(B, Sq, Hq, Dh), 0, 2, 1, 3)
        k = jnp.repeat(k_cache[:, :, Sk - W:, :], rep, axis=1)
        v = jnp.repeat(v_cache[:, :, Sk - W:, :], rep, axis=1)
        scores = jnp.einsum("bhqd,bhkd->bhqk", q, k) * (Dh ** -0.5)
        p = _softmax(scores, axis=-1)
        o = jnp.einsum("bhqk,bhkd->bhqd", p, v)
        return (lambda x, *d: x.transpose(*d))(o, 0, 2, 1, 3).reshape(B, Sq, Hq * Dh) @ wo

    def _B_ref(x, w_r, w_gate, w_up, w_down):
        B, S, D = x.shape
        C = 1
        r = x @ w_r
        idx = jnp.argsort(-r, axis=-1)[:, :C]
        idx_e = jnp.repeat(idx.reshape(B, C, 1), D, axis=2)
        x_sel = jnp.take_along_axis(x, idx_e, axis=1)
        g = _silu(x_sel @ w_gate)
        u = x_sel @ w_up
        y = (g * u) @ w_down
        r_sel = _sigmoid(jnp.take_along_axis(r, idx, axis=1))
        y = y * r_sel.reshape(B, C, 1)
        b_off = (jnp.arange(B) * S).reshape(B, 1)
        flat_idx = (idx + b_off).reshape(B * C)
        zero = (x * 0.0).reshape(B * S, D)
        upd = _scatter_add(zero, flat_idx, y.reshape(B * C, D), axis=0)
        return x + upd.reshape(B, S, D)

    x = A_x
    h = x + _A_ref(_layernorm(x, axis=-1), A_k_cache, A_v_cache, A_wq, A_wo)
    h2 = h + _B_ref(_layernorm(h, axis=-1), B_w_r, B_w_gate, B_w_up, B_w_down)
    return h2
```

```python
import jax
import jax.numpy as jnp
from jax import lax
import jax.experimental.pallas as pl
import jax.experimental.pallas.tpu as pltpu

EPS = 1e-5
LOOK = 3
SLAB = 48
RUN = 8
ROW = 16
UP_CHUNKS = (44, 16)
DOWN_CHUNKS = (14, 8, 4, 2, 1, 1)


def _layernorm(x):
    m = jnp.mean(x, axis=-1, keepdims=True)
    d = x - m
    v = jnp.mean(d * d, axis=-1, keepdims=True)
    return d / jnp.sqrt(v + EPS)


def _tile_pairs(w):
    r, c = w.shape
    return w.reshape(r // 8, 8, c // 128, 128).transpose(0, 2, 1, 3).reshape(-1, 16, 128)


def _split(items, sizes):
    out, start = [], 0
    for n in sizes:
        out.append(items[start:start + n])
        start += n
    assert start == len(items)
    return out


def _kernel(x_hbm, k_hbm, v_hbm, wq_hbm, wo_hbm, wr_hbm, wg_hbm, wu_hbm, wd_hbm, o_ref,
            x_s, wr_s, wq_s, wo_s, wg_s, wu_s, wd_s, k_s, v_s, q_s, p_s, inv_s, acc_s, col_s,
            sem_k, sem_v, sem_w, sem_u, sem_d):
    f32, bf16 = jnp.float32, jnp.bfloat16
    H, n_slab, _, W = k_s.shape
    Dh = n_slab * SLAB
    first = k_hbm.shape[-1] - W
    D = x_hbm.shape[-1]
    F = col_s.shape[0]

    def loop(lo, hi, body):
        lax.fori_loop(lo, hi, lambda i, _: body(i), None)

    def done(buf, sem):
        pltpu.make_async_copy(buf, buf, sem).wait()

    def kv_start(src, dst, sem, h):
        def body(u):
            c = pl.multiple_of(u * 1024, 1024)
            for q in range(0, n_slab, 2):
                for r in range(SLAB // 8):
                    rows = (h, pl.ds(q, 2), pl.ds(r * 8, 8))
                    pltpu.make_async_copy(src.at[(*rows, pl.ds(first + c, 1024))],
                                          dst.at[(*rows, pl.ds(c, 1024))],
                                          sem.at[h]).start(priority=r % 2)
        loop(0, W // 1024, body)

    def wq_copy(n):
        idx = (pl.ds(pl.multiple_of((n // 3) * 8, 8), 8),
               pl.ds(pl.multiple_of((n % 3) * 2048, 2048), 2048))
        return pltpu.make_async_copy(wq_hbm.at[idx], wq_s.at[idx], sem_w.at[0])

    def run_copy(src, dst, sem, n):
        return pltpu.make_async_copy(src.at[pl.ds(n * RUN, RUN)], dst.at[pl.ds(n * RUN, RUN)], sem)

    def wo_copy(n):
        return run_copy(wo_hbm, wo_s, sem_w.at[1], n)

    n_row = wo_s.shape[0] // (RUN * ROW)

    def proj_start(copy, i, thread0=0):
        for t in range(2):
            s = 2 * i + t
            n = (s % n_row) * ROW + (s // n_row) * 2
            copy(n + t).start(priority=thread0)
            copy(n + 1 - t).start(priority=1)

    n_proj = n_row * ROW // 4
    n_ffn = wd_s.shape[0] // RUN
    segs = [ROW // 2 * r + j for j in range(ROW // 2) for r in range(pl.cdiv(n_ffn, ROW))
            if ROW * r + 2 * j < n_ffn]
    ffn_order = [(2 * m + ((s & 1) ^ th), th) for s, m in enumerate(segs) for th in range(2)]
    up_chunks = _split(ffn_order, UP_CHUNKS)
    down_chunks = ([c for c in ffn_order if c[1] == 0],
                   *_split([c for c in ffn_order if c[1] == 1], DOWN_CHUNKS))

    def wg_start():
        for n, th in ffn_order:
            run_copy(wg_hbm, wg_s, sem_w.at[2], n).start(priority=th)

    def wu_start():
        for c, chunk in enumerate(up_chunks):
            for n, th in chunk:
                run_copy(wu_hbm, wu_s, sem_u.at[c], n).start(priority=th)

    def wd_start():
        which = {item: c for c, chunk in enumerate(down_chunks) for item in chunk}
        for n, th in ffn_order:
            run_copy(wd_hbm, wd_s, sem_d.at[which[n, th]], n).start(priority=th)

    x_cp = pltpu.make_async_copy(x_hbm, x_s, sem_w.at[3])
    wr_cp = pltpu.make_async_copy(wr_hbm, wr_s, sem_w.at[4])

    loop(0, 6, lambda i: proj_start(wq_copy, i, thread0=1))
    loop(6, n_proj, lambda i: proj_start(wq_copy, i))
    x_cp.start()
    wr_cp.start()
    loop(0, LOOK, lambda h: kv_start(k_hbm, k_s, sem_k, h))

    x_cp.wait()
    x = x_s[0].astype(f32)
    xn = jnp.broadcast_to(_layernorm(x), (8, D)).astype(bf16)
    done(wq_s, sem_w.at[0])
    per_head = Dh * W // (4 * RUN * 2048)

    def k_step(h):
        @pl.when(h + LOOK < H)
        def _():
            kv_start(k_hbm, k_s, sem_k, h + LOOK)

        @pl.when(h + LOOK >= H)
        def _():
            lo = (h + LOOK - H) * per_head
            loop(lo, lo + per_head, lambda i: proj_start(wo_copy, i))

        @pl.when(h % 2 == 0)
        def _():
            col = pl.multiple_of((h // 2) * (2 * Dh), 128)
            q2 = jnp.dot(xn, wq_s[:, pl.ds(col, 2 * Dh)], preferred_element_type=f32)
            q_s[0] = q2[:, :Dh]
            q_s[1] = q2[:, Dh:]

        done(k_s.at[h], sem_k.at[h])
        s = jnp.dot(q_s[h % 2].astype(bf16), k_s[h].reshape(Dh, W),
                    preferred_element_type=f32) * Dh ** -0.5
        e = jnp.exp(s - jnp.max(s, axis=-1, keepdims=True))
        p_s[h] = e
        inv_s[h] = jnp.broadcast_to(1.0 / jnp.sum(e, axis=-1, keepdims=True), (8, 128))

    loop(0, H, k_step)
    loop(LOOK * per_head, n_proj, lambda i: proj_start(wo_copy, i))
    loop(0, LOOK, lambda h: kv_start(v_hbm, v_s, sem_v, h))

    acc_s[...] = jnp.zeros_like(acc_s)
    done(wo_s, sem_w.at[1])
    n_d = D // 128

    def v_step(h):
        @pl.when(h + LOOK < H)
        def _():
            kv_start(v_hbm, v_s, sem_v, h + LOOK)

        pl.when(h + LOOK == H)(wg_start)
        pl.when(h + LOOK == H + 1)(wu_start)

        done(v_s.at[h], sem_v.at[h])
        inv = inv_s[h][:, :1]
        acc = [acc_s[c] for c in range(n_d)]
        for r in range(Dh // 16):
            slab, r0 = divmod(r * 16, SLAB)
            a0 = jnp.zeros((8, 128), f32)
            a1 = jnp.zeros((8, 128), f32)
            for j in range(0, W, 128):
                pp = p_s[h, :, j:j + 128]
                vv = v_s[h, slab, r0:r0 + 16, j:j + 128].astype(f32)
                a0 = a0 + vv[:8] * pp
                a1 = a1 + vv[8:] * pp
            o = [jnp.sum(a, axis=-1, keepdims=True) * inv for a in (a0, a1)]
            for b in range(n_d):
                ww = wo_s[(h * (Dh // 16) + r) * n_d + b].astype(f32)
                for t in range(2):
                    g, c = divmod(2 * b + t, n_d)
                    acc[c] = acc[c] + ww[8 * t:8 * t + 8] * o[g]
        for c in range(n_d):
            acc_s[c] = acc[c]

    loop(0, H, v_step)
    wd_start()

    def set_columns(row):
        for b in range(0, row.shape[1], 128):
            col_s[b:b + 128, :] = jnp.broadcast_to(row[:, b:b + 128], (128, 128)).T

    def gemv(acc, w_s, copies):
        acc = list(acc)
        for n, _ in copies:
            for b in range(n * RUN, (n + 1) * RUN):
                ww = w_s[b].astype(f32)
                for t in range(2):
                    g, c = divmod(2 * b + t, len(acc))
                    acc[c] = acc[c] + ww[8 * t:8 * t + 8] * col_s[8 * g:8 * g + 8, :]
        return acc

    def fold(acc):
        return jnp.concatenate([jnp.sum(a, axis=0, keepdims=True) for a in acc], axis=1)

    def zeros(n):
        return [jnp.zeros((8, 128), f32)] * (n // 128)

    hres = x + fold([acc_s[c] for c in range(n_d)])
    hn = _layernorm(hres)
    wr_cp.wait()
    wr = wr_s[...].astype(f32).reshape(1, D)
    gate = jax.nn.sigmoid(jnp.sum(hn * wr, axis=-1, keepdims=True))
    set_columns(hn)

    done(wg_s, sem_w.at[2])
    g = fold(gemv(zeros(F), wg_s, ffn_order))
    g = g * jax.nn.sigmoid(g)
    acc = zeros(F)
    for c, chunk in enumerate(up_chunks):
        for n, _ in chunk:
            run_copy(wu_hbm, wu_s, sem_u.at[c], n).wait()
        acc = gemv(acc, wu_s, chunk)
    set_columns(g * fold(acc))

    acc = zeros(D)
    for c, chunk in enumerate(down_chunks):
        for n, _ in chunk:
            run_copy(wd_hbm, wd_s, sem_d.at[c], n).wait()
        acc = gemv(acc, wd_s, chunk)
    o_ref[0] = (hres + hn + fold(acc) * gate).astype(o_ref.dtype)


@jax.jit
def pallas_sequential_preLN__sliding_block_cached__moe_arch_mod__decode_kernel(
    A_x: jax.Array,
    A_k_cache: jax.Array,
    A_v_cache: jax.Array,
    A_wq: jax.Array,
    A_wo: jax.Array,
    B_x: jax.Array,
    B_w_r: jax.Array,
    B_w_gate: jax.Array,
    B_w_up: jax.Array,
    B_w_down: jax.Array,
):
    del B_x
    _, H, Sk, Dh = A_k_cache.shape
    D = A_x.shape[-1]
    F = B_w_gate.shape[-1]
    W = min(4096, max(256, Sk // 4))
    kt = jnp.transpose(A_k_cache, (0, 1, 3, 2)).reshape(H, Dh // SLAB, SLAB, Sk)
    vt = jnp.transpose(A_v_cache, (0, 1, 3, 2)).reshape(H, Dh // SLAB, SLAB, Sk)
    wo, wg, wu, wd = (_tile_pairs(w) for w in (A_wo, B_w_gate, B_w_up, B_w_down))
    like = lambda a: pltpu.VMEM(a.shape, a.dtype)
    return pl.pallas_call(
        _kernel,
        out_shape=jax.ShapeDtypeStruct(A_x.shape, A_x.dtype),
        in_specs=[pl.BlockSpec(memory_space=pl.ANY)] * 9,
        scratch_shapes=[
            like(A_x), like(B_w_r), like(A_wq), like(wo), like(wg), like(wu), like(wd),
            pltpu.VMEM((H, Dh // SLAB, SLAB, W), A_k_cache.dtype),
            pltpu.VMEM((H, Dh // SLAB, SLAB, W), A_v_cache.dtype),
            pltpu.VMEM((2, 8, Dh), jnp.float32),
            pltpu.VMEM((H, 8, W), jnp.float32),
            pltpu.VMEM((H, 8, 128), jnp.float32),
            pltpu.VMEM((D // 128, 8, 128), jnp.float32),
            pltpu.VMEM((F, 128), jnp.float32),
            pltpu.SemaphoreType.DMA((H,)),
            pltpu.SemaphoreType.DMA((H,)),
            pltpu.SemaphoreType.DMA((5,)),
            pltpu.SemaphoreType.DMA((len(UP_CHUNKS),)),
            pltpu.SemaphoreType.DMA((len(DOWN_CHUNKS) + 1,)),
        ],
        compiler_params=pltpu.CompilerParams(
            vmem_limit_bytes=126 * 2**20, disable_bounds_checks=True,
            disable_semaphore_checks=True),
    )(A_x, kt, vt, A_wq, wo, B_w_r, wg, wu, wd)
```

```python
import jax
import jax.numpy as jnp
from jax import lax
import jax.experimental.pallas as pl
import jax.experimental.pallas.tpu as pltpu

EPS = 1e-5
LOOK = 2
KV_ROWS, KV_COLS = 32, 512
PROJ_STEPS = 15
PROJ_ROWS = ((0, 3), (3, 4), (7, 4), (11, 4))
PROJ_AHEAD = 13
FFN_STEPS = 4
UP_CHUNKS = (40, 20)
DOWN_CHUNKS = (28, 16, 8, 4, 2, 1, 1)


def _layernorm(x):
    m = jnp.mean(x, axis=-1, keepdims=True)
    d = x - m
    v = jnp.mean(d * d, axis=-1, keepdims=True)
    return d / jnp.sqrt(v + EPS)


def _tile_pairs(w, steps):
    r, c = w.shape
    return w.reshape(r // 8, 8, c // 128, 128).transpose(0, 2, 1, 3).reshape(steps, -1, 16, 128)


def _ranges(sizes):
    out, lo = [], 0
    for n in sizes:
        out.append((lo, lo + n))
        lo += n
    return out


def _kernel(x_hbm, k_hbm, v_hbm, wq_hbm, wo_hbm, wr_hbm, wg_hbm, wu_hbm, wd_hbm, o_ref,
            x_s, wr_s, proj_s, ffn_s, kv_s, q_s, p_s, inv_s, acc_s, col_s,
            sem_k, sem_v, sem_w, sem_g, sem_u, sem_d):
    f32, bf16 = jnp.float32, jnp.bfloat16
    wq_s, wo_s = proj_s.at[0], proj_s.at[1]
    wg_s, wu_s, wd_s = ffn_s.at[0], ffn_s.at[1], ffn_s.at[2]
    k_s, v_s = kv_s.at[0], kv_s.at[1]
    _, H, Dh, W = kv_s.shape
    first = k_hbm.shape[-1] - W
    D = x_hbm.shape[-1]
    F = col_s.shape[0]
    n_d = D // 128

    def loop(lo, hi, body):
        lax.fori_loop(lo, hi, lambda i, _: body(i), None)

    def done(buf, sem):
        pltpu.make_async_copy(buf, buf, sem).wait()

    K, V = (k_hbm, k_s, sem_k), (v_hbm, v_s, sem_v)
    WQ, WO = (wq_hbm, wq_s, sem_w.at[0]), (wo_hbm, wo_s, sem_w.at[1])
    sweep = Dh // KV_ROWS // 2
    n_kv = sweep * (W // KV_COLS)

    def kv_start(arr, h, u, r, thread):
        src, dst, sem = arr
        r, c = (2 * r + thread) * KV_ROWS, u * KV_COLS
        if not isinstance(r, int):
            r = pl.multiple_of(r, KV_ROWS)
        c = pl.multiple_of(c, KV_COLS)
        pltpu.make_async_copy(src.at[h, pl.ds(r, KV_ROWS), pl.ds(first + c, KV_COLS)],
                              dst.at[h, pl.ds(r, KV_ROWS), pl.ds(c, KV_COLS)],
                              sem.at[h]).start(priority=thread)

    def head_start(arr0, h0, arr1, h1):
        def body(u):
            for r in range(sweep):
                kv_start(arr0, h0, u, r, 0)
                kv_start(arr1, h1, u, r, 1)
        loop(0, W // KV_COLS, body)

    def proj_start(arr, u, i):
        src, dst, sem = arr
        idx = (pl.ds(*PROJ_ROWS[i]), pl.ds(2 * u, 2))
        pltpu.make_async_copy(src.at[idx], dst.at[idx], sem).start(priority=i % 2)

    def proj_sweep(arr0, u0, arr1, u1):
        for i in (0, 2):
            proj_start(arr0, u0, i)
            proj_start(arr1, u1, i + 1)

    n_ffn = wd_s.shape[1] // 2
    up, down = _ranges(UP_CHUNKS), _ranges(DOWN_CHUNKS)
    FFN = {"g": (wg_hbm, wg_s, sem_g, up), "u": (wu_hbm, wu_s, sem_u, up),
           "d": (wd_hbm, wd_s, sem_d, down)}

    def ffn_start(name, u, thread):
        src, dst, sems, chunks = FFN[name]
        c = next(i for i, (lo, hi) in enumerate(chunks) if lo <= u < hi)
        idx = (slice(None), pl.ds(2 * u, 2))
        pltpu.make_async_copy(src.at[idx], dst.at[idx], sems.at[c]).start(priority=thread)

    order = [(a, u) for u in range(n_ffn) for a in "gu"] + [("d", u) for u in range(n_ffn)]
    paired = len(order) - n_kv
    ffn0 = order[0:paired:2]
    ffn1 = order[1:paired:2] + order[paired:]

    def ffn_part(part):
        n = len(ffn0) // 3
        for i in range(part * n, (part + 1) * n):
            ffn_start(*ffn0[i], 0)
            ffn_start(*ffn1[n_kv + i], 1)

    x_cp = pltpu.make_async_copy(x_hbm, x_s, sem_w.at[2])
    wr_cp = pltpu.make_async_copy(wr_hbm, wr_s, sem_w.at[3])

    n_u = wq_s.shape[1] // 2
    both = n_u - PROJ_AHEAD
    for u in range(PROJ_AHEAD):
        proj_start(WQ, u, 1)
        proj_start(WQ, u, 3)
    loop(0, both, lambda u: proj_sweep(WQ, u, WQ, u + PROJ_AHEAD))
    x_cp.start()
    wr_cp.start()
    loop(both, n_u, lambda u: proj_sweep(WQ, u, WO, u - both))
    loop(0, both, lambda u: proj_sweep(WO, u, WO, u + PROJ_AHEAD))

    def wo_to_k(u):
        for t in range(2):
            j = 2 * (u - both) + t
            proj_start(WO, u, 2 * t)
            pl.when(j < n_kv)(lambda j=j: kv_start(K, 0, j // sweep, j % sweep, 1))

    loop(both, n_u, wo_to_k)
    loop(0, LOOK, lambda h: head_start(K, h, K, h + 1))

    def set_columns(row):
        for b in range(0, row.shape[1], 128):
            col_s[b:b + 128, :] = jnp.broadcast_to(row[:, b:b + 128], (128, 128)).T

    def zeros(n):
        return [jnp.zeros((8, 128), f32)] * (n // 128)

    def fold(acc):
        return jnp.concatenate([jnp.sum(a, axis=0, keepdims=True) for a in acc], axis=1)

    def proj_block(ref, b):
        n = ref.shape[1]
        assert n & (n - 1) == 0
        return ref[b >> (n.bit_length() - 1), b & (n - 1)].astype(f32)

    x_cp.wait()
    x = x_s[0].astype(f32)
    set_columns(_layernorm(x))
    done(wq_s, sem_w.at[0])

    def k_step(h):
        j = h + LOOK
        pl.when(j < H - 1)(lambda: head_start(K, j, K, j + 1))
        pl.when(j == H - 1)(lambda: head_start(K, H - 1, V, 0))
        pl.when(j >= H)(lambda: head_start(V, j - H, V, j - H + 1))

        @pl.when(h % 4 == 0)
        def _():
            acc = list(zeros(4 * Dh))
            per_row = H * Dh // 256
            for g in range(D // 8):
                xc = col_s[8 * g:8 * g + 8, :]
                for i in range(len(acc) // 2):
                    ww = proj_block(wq_s, per_row * g + i + (h // 4) * (len(acc) // 2))
                    acc[2 * i] = acc[2 * i] + ww[:8] * xc
                    acc[2 * i + 1] = acc[2 * i + 1] + ww[8:] * xc
            q4 = jnp.broadcast_to(fold(acc), (8, 4 * Dh))
            for i in range(4):
                q_s[i] = q4[:, i * Dh:(i + 1) * Dh]

        done(k_s.at[h], sem_k.at[h])
        s = jnp.dot(q_s[h % 4].astype(bf16), k_s[h], preferred_element_type=f32) * Dh ** -0.5
        e = jnp.exp(s - jnp.max(s, axis=-1, keepdims=True))
        p_s[h] = e
        inv_s[h] = jnp.broadcast_to(1.0 / jnp.sum(e, axis=-1, keepdims=True), (8, 128))

    loop(0, H, k_step)

    acc_s[...] = jnp.zeros_like(acc_s)
    done(wo_s, sem_w.at[1])

    def v_to_ffn(j):
        kv_start(V, H - 1, j // sweep, j % sweep, 0)
        idx = (slice(None), pl.ds(2 * j, 2))
        pltpu.make_async_copy(wu_hbm.at[idx], wu_s.at[idx], sem_u.at[0]).start(priority=1)

    def v_step(h):
        j = h + LOOK
        pl.when(j < H - 1)(lambda: head_start(V, j, V, j + 1))
        pl.when(j == H - 1)(lambda: loop(0, n_kv, v_to_ffn))
        pl.when(j == H)(lambda: ffn_part(0))
        pl.when(j == H + 1)(lambda: ffn_part(1))

        done(v_s.at[h], sem_v.at[h])
        inv = inv_s[h][:, :1]
        acc = [acc_s[c] for c in range(n_d)]
        for r in range(Dh // 16):
            a0 = jnp.zeros((8, 128), f32)
            a1 = jnp.zeros((8, 128), f32)
            for c in range(0, W, 128):
                pp = p_s[h, :, c:c + 128]
                vv = v_s[h, r * 16:(r + 1) * 16, c:c + 128].astype(f32)
                a0 = a0 + vv[:8] * pp
                a1 = a1 + vv[8:] * pp
            o = [jnp.sum(a, axis=-1, keepdims=True) * inv for a in (a0, a1)]
            for b in range(n_d):
                ww = proj_block(wo_s, (h * (Dh // 16) + r) * n_d + b)
                for t in range(2):
                    g, c = divmod(2 * b + t, n_d)
                    acc[c] = acc[c] + ww[8 * t:8 * t + 8] * o[g]
        for c in range(n_d):
            acc_s[c] = acc[c]

    loop(0, H, v_step)
    ffn_part(2)

    def gemv(acc, w_s, sem, lo, hi):
        done(w_s.at[:, 2 * lo:2 * hi], sem)
        acc = list(acc)
        for b in range(2 * lo, 2 * hi):
            for s in range(w_s.shape[0]):
                ww = w_s[s, b].astype(f32)
                for t in range(2):
                    g, c = divmod(2 * (s * w_s.shape[1] + b) + t, len(acc))
                    acc[c] = acc[c] + ww[8 * t:8 * t + 8] * col_s[8 * g:8 * g + 8, :]
        return acc

    hres = x + fold([acc_s[c] for c in range(n_d)])
    hn = _layernorm(hres)
    wr_cp.wait()
    wr = wr_s[...].astype(f32).reshape(1, D)
    gate = jax.nn.sigmoid(jnp.sum(hn * wr, axis=-1, keepdims=True))
    set_columns(hn)

    g, u = zeros(F), zeros(F)
    for c, (lo, hi) in enumerate(up):
        g = gemv(g, wg_s, sem_g.at[c], lo, hi)
        u = gemv(u, wu_s, sem_u.at[c], lo, hi)
    g = fold(g)
    set_columns(g * jax.nn.sigmoid(g) * fold(u))

    y = zeros(D)
    for c, (lo, hi) in enumerate(down):
        y = gemv(y, wd_s, sem_d.at[c], lo, hi)
    o_ref[0] = (hres + hn + fold(y) * gate).astype(o_ref.dtype)


@jax.jit
def pallas_sequential_preLN__sliding_block_cached__moe_arch_mod__decode_kernel(
    A_x: jax.Array,
    A_k_cache: jax.Array,
    A_v_cache: jax.Array,
    A_wq: jax.Array,
    A_wo: jax.Array,
    B_x: jax.Array,
    B_w_r: jax.Array,
    B_w_gate: jax.Array,
    B_w_up: jax.Array,
    B_w_down: jax.Array,
):
    del B_x
    _, H, Sk, Dh = A_k_cache.shape
    D = A_x.shape[-1]
    F = B_w_gate.shape[-1]
    W = min(4096, max(256, Sk // 4))
    kt = jnp.transpose(A_k_cache, (0, 1, 3, 2)).reshape(H, Dh, Sk)
    vt = jnp.transpose(A_v_cache, (0, 1, 3, 2)).reshape(H, Dh, Sk)
    wq, wo = (_tile_pairs(w, PROJ_STEPS) for w in (A_wq, A_wo))
    wg, wu, wd = (_tile_pairs(w, FFN_STEPS) for w in (B_w_gate, B_w_up, B_w_down))
    return pl.pallas_call(
        _kernel,
        out_shape=jax.ShapeDtypeStruct(A_x.shape, A_x.dtype),
        in_specs=[pl.BlockSpec(memory_space=pl.ANY)] * 9,
        scratch_shapes=[
            pltpu.VMEM(A_x.shape, A_x.dtype),
            pltpu.VMEM(B_w_r.shape, B_w_r.dtype),
            pltpu.VMEM((2, *wq.shape), wq.dtype),
            pltpu.VMEM((3, *wg.shape), wg.dtype),
            pltpu.VMEM((2, H, Dh, W), kt.dtype),
            pltpu.VMEM((4, 8, Dh), jnp.float32),
            pltpu.VMEM((H, 8, W), jnp.float32),
            pltpu.VMEM((H, 8, 128), jnp.float32),
            pltpu.VMEM((D // 128, 8, 128), jnp.float32),
            pltpu.VMEM((F, 128), jnp.float32),
            pltpu.SemaphoreType.DMA((H,)),
            pltpu.SemaphoreType.DMA((H,)),
            pltpu.SemaphoreType.DMA((4,)),
            pltpu.SemaphoreType.DMA((len(UP_CHUNKS),)),
            pltpu.SemaphoreType.DMA((len(UP_CHUNKS),)),
            pltpu.SemaphoreType.DMA((len(DOWN_CHUNKS),)),
        ],
        compiler_params=pltpu.CompilerParams(
            vmem_limit_bytes=126 * 2**20, disable_bounds_checks=True,
            disable_semaphore_checks=True),
    )(A_x, kt, vt, wq, wo, B_w_r, wg, wu, wd)
```

```python
import jax
import jax.numpy as jnp
from jax import lax
import jax.experimental.pallas as pl
import jax.experimental.pallas.tpu as pltpu

EPS = 1e-5
LOOK = 2
KV_ROWS, KV_COLS = 32, 512
KV_AHEAD = 9
PROJ_STEPS = 15
PROJ_ROWS = ((0, 3), (3, 4), (7, 4), (11, 4))
PROJ_AHEAD = 13
FFN_STEPS = 4
UP_CHUNKS = (40, 20)
DOWN_CHUNKS = (28, 16, 8, 4, 2, 1, 1)


def _layernorm(x):
    m = jnp.mean(x, axis=-1, keepdims=True)
    d = x - m
    v = jnp.mean(d * d, axis=-1, keepdims=True)
    return d / jnp.sqrt(v + EPS)


def _tile_pairs(w, steps):
    r, c = w.shape
    return w.reshape(r // 8, 8, c // 128, 128).transpose(0, 2, 1, 3).reshape(steps, -1, 16, 128)


def _ranges(sizes):
    out, lo = [], 0
    for n in sizes:
        out.append((lo, lo + n))
        lo += n
    return out


def _kernel(x_hbm, k_hbm, v_hbm, wq_hbm, wo_hbm, wr_hbm, wg_hbm, wu_hbm, wd_hbm, o_ref,
            x_s, wr_s, proj_s, ffn_s, kv_s, q_s, p_s, inv_s, acc_s, col_s,
            sem_k, sem_v, sem_w, sem_g, sem_u, sem_d):
    f32, bf16 = jnp.float32, jnp.bfloat16
    wq_s, wo_s = proj_s.at[0], proj_s.at[1]
    wg_s, wu_s, wd_s = ffn_s.at[0], ffn_s.at[1], ffn_s.at[2]
    k_s, v_s = kv_s.at[0], kv_s.at[1]
    _, H, Dh, W = kv_s.shape
    first = k_hbm.shape[-1] - W
    D = x_hbm.shape[-1]
    F = col_s.shape[0]
    n_d = D // 128

    def loop(lo, hi, body):
        lax.fori_loop(lo, hi, lambda i, _: body(i), None)

    def done(buf, sem):
        pltpu.make_async_copy(buf, buf, sem).wait()

    K, V = (k_hbm, k_s, sem_k), (v_hbm, v_s, sem_v)
    WQ, WO = (wq_hbm, wq_s, sem_w.at[0]), (wo_hbm, wo_s, sem_w.at[1])
    pairs = Dh // KV_ROWS // 2
    per_head = W // KV_COLS
    n_sweep = H * per_head
    ahead = KV_AHEAD * pairs

    def kv_start(arr, s, r, thread):
        src, dst, sem = arr
        h = s >> (per_head.bit_length() - 1)
        c = pl.multiple_of((s & (per_head - 1)) * KV_COLS, KV_COLS)
        r = (2 * r + thread) * KV_ROWS
        if not isinstance(r, int):
            r = pl.multiple_of(r, KV_ROWS)
        pltpu.make_async_copy(src.at[h, pl.ds(r, KV_ROWS), pl.ds(first + c, KV_COLS)],
                              dst.at[h, pl.ds(r, KV_ROWS), pl.ds(c, KV_COLS)],
                              sem.at[h]).start(priority=thread)

    def kv_sweep(arr0, s0, arr1, s1):
        for r in range(pairs):
            kv_start(arr0, s0, r, 0)
            kv_start(arr1, s1, r, 1)

    def proj_start(arr, u, i):
        src, dst, sem = arr
        idx = (pl.ds(*PROJ_ROWS[i]), pl.ds(2 * u, 2))
        pltpu.make_async_copy(src.at[idx], dst.at[idx], sem).start(priority=i % 2)

    def proj_sweep(arr0, u0, arr1, u1):
        for i in (0, 2):
            proj_start(arr0, u0, i)
            proj_start(arr1, u1, i + 1)

    n_ffn = wd_s.shape[1] // 2
    up, down = _ranges(UP_CHUNKS), _ranges(DOWN_CHUNKS)
    FFN = {"g": (wg_hbm, wg_s, sem_g, up), "u": (wu_hbm, wu_s, sem_u, up),
           "d": (wd_hbm, wd_s, sem_d, down)}

    def ffn_start(name, u, thread):
        src, dst, sems, chunks = FFN[name]
        c = next(i for i, (lo, hi) in enumerate(chunks) if lo <= u < hi)
        idx = (slice(None), pl.ds(2 * u, 2))
        pltpu.make_async_copy(src.at[idx], dst.at[idx], sems.at[c]).start(priority=thread)

    order = [(a, u) for u in range(n_ffn) for a in "gu"] + [("d", u) for u in range(n_ffn)]
    paired = (len(order) - ahead) // 2 * 2
    ffn0 = order[0:paired:2]
    ffn1 = order[1:paired:2] + order[paired:]

    def ffn_part(part):
        n = pl.cdiv(len(ffn1) - ahead, 3)
        for i in range(part * n, min((part + 1) * n, len(ffn1) - ahead)):
            if i < len(ffn0):
                ffn_start(*ffn0[i], 0)
            ffn_start(*ffn1[ahead + i], 1)

    def v_to_ffn(s):
        for r in range(pairs):
            kv_start(V, s - n_sweep, r, 0)
            idx = (slice(None), pl.ds(2 * ((s + KV_AHEAD - 2 * n_sweep) * pairs + r), 2))
            pltpu.make_async_copy(wu_hbm.at[idx], wu_s.at[idx], sem_u.at[0]).start(priority=1)

    assert ffn1[:ahead] == [("u", u) for u in range(ahead)] and up[0][1] >= ahead
    stages = (
        (0, n_sweep - KV_AHEAD, lambda s: kv_sweep(K, s, K, s + KV_AHEAD)),
        (n_sweep - KV_AHEAD, n_sweep, lambda s: kv_sweep(K, s, V, s + KV_AHEAD - n_sweep)),
        (n_sweep, 2 * n_sweep - KV_AHEAD,
         lambda s: kv_sweep(V, s - n_sweep, V, s + KV_AHEAD - n_sweep)),
        (2 * n_sweep - KV_AHEAD, 2 * n_sweep, v_to_ffn))

    def head_start(j, which):
        for lo, hi, body in which:
            loop(jnp.clip(j * per_head, lo, hi), jnp.clip((j + 1) * per_head, lo, hi), body)

    x_cp = pltpu.make_async_copy(x_hbm, x_s, sem_w.at[2])
    wr_cp = pltpu.make_async_copy(wr_hbm, wr_s, sem_w.at[3])

    n_u = wq_s.shape[1] // 2
    both = n_u - PROJ_AHEAD
    for u in range(PROJ_AHEAD):
        proj_start(WQ, u, 1)
        proj_start(WQ, u, 3)
    loop(0, both, lambda u: proj_sweep(WQ, u, WQ, u + PROJ_AHEAD))
    x_cp.start()
    wr_cp.start()
    loop(both, n_u, lambda u: proj_sweep(WQ, u, WO, u - both))
    loop(0, both, lambda u: proj_sweep(WO, u, WO, u + PROJ_AHEAD))

    def k_first(j):
        kv_start(K, j // pairs, j % pairs, 1)

    def wo_to_k(u):
        for t in range(2):
            proj_start(WO, u, 2 * t)
            k_first(2 * (u - both) + t)

    loop(both, n_u, wo_to_k)
    loop(2 * PROJ_AHEAD, ahead, k_first)
    loop(0, LOOK * per_head, stages[0][2])

    def set_columns(row):
        for b in range(0, row.shape[1], 128):
            col_s[b:b + 128, :] = jnp.broadcast_to(row[:, b:b + 128], (128, 128)).T

    def zeros(n):
        return [jnp.zeros((8, 128), f32)] * (n // 128)

    def fold(acc):
        return jnp.concatenate([jnp.sum(a, axis=0, keepdims=True) for a in acc], axis=1)

    def proj_block(ref, b):
        n = ref.shape[1]
        assert n & (n - 1) == 0
        return ref[b >> (n.bit_length() - 1), b & (n - 1)].astype(f32)

    x_cp.wait()
    x = x_s[0].astype(f32)
    set_columns(_layernorm(x))
    done(wq_s, sem_w.at[0])

    def k_step(h):
        head_start(h + LOOK, stages[:3])

        @pl.when(h % 4 == 0)
        def _():
            acc = list(zeros(4 * Dh))
            per_row = H * Dh // 256
            for g in range(D // 8):
                xc = col_s[8 * g:8 * g + 8, :]
                for i in range(len(acc) // 2):
                    ww = proj_block(wq_s, per_row * g + i + (h // 4) * (len(acc) // 2))
                    acc[2 * i] = acc[2 * i] + ww[:8] * xc
                    acc[2 * i + 1] = acc[2 * i + 1] + ww[8:] * xc
            q4 = jnp.broadcast_to(fold(acc), (8, 4 * Dh))
            for i in range(4):
                q_s[i] = q4[:, i * Dh:(i + 1) * Dh]

        done(k_s.at[h], sem_k.at[h])
        s = jnp.dot(q_s[h % 4].astype(bf16), k_s[h], preferred_element_type=f32) * Dh ** -0.5
        e = jnp.exp(s - jnp.max(s, axis=-1, keepdims=True))
        p_s[h] = e
        inv_s[h] = jnp.broadcast_to(1.0 / jnp.sum(e, axis=-1, keepdims=True), (8, 128))

    loop(0, H, k_step)

    acc_s[...] = jnp.zeros_like(acc_s)
    done(wo_s, sem_w.at[1])

    def v_step(h):
        head_start(H + h + LOOK, stages[2:])
        pl.when(h + LOOK == H)(lambda: ffn_part(0))
        pl.when(h + LOOK == H + 1)(lambda: ffn_part(1))

        done(v_s.at[h], sem_v.at[h])
        inv = inv_s[h][:, :1]
        acc = [acc_s[c] for c in range(n_d)]
        for r in range(Dh // 16):
            a0 = jnp.zeros((8, 128), f32)
            a1 = jnp.zeros((8, 128), f32)
            for c in range(0, W, 128):
                pp = p_s[h, :, c:c + 128]
                vv = v_s[h, r * 16:(r + 1) * 16, c:c + 128].astype(f32)
                a0 = a0 + vv[:8] * pp
                a1 = a1 + vv[8:] * pp
            o = [jnp.sum(a, axis=-1, keepdims=True) * inv for a in (a0, a1)]
            for b in range(n_d):
                ww = proj_block(wo_s, (h * (Dh // 16) + r) * n_d + b)
                for t in range(2):
                    g, c = divmod(2 * b + t, n_d)
                    acc[c] = acc[c] + ww[8 * t:8 * t + 8] * o[g]
        for c in range(n_d):
            acc_s[c] = acc[c]

    loop(0, H, v_step)
    ffn_part(2)

    def gemv(acc, w_s, sem, lo, hi):
        done(w_s.at[:, 2 * lo:2 * hi], sem)
        acc = list(acc)
        for b in range(2 * lo, 2 * hi):
            for s in range(w_s.shape[0]):
                ww = w_s[s, b].astype(f32)
                for t in range(2):
                    g, c = divmod(2 * (s * w_s.shape[1] + b) + t, len(acc))
                    acc[c] = acc[c] + ww[8 * t:8 * t + 8] * col_s[8 * g:8 * g + 8, :]
        return acc

    hres = x + fold([acc_s[c] for c in range(n_d)])
    hn = _layernorm(hres)
    wr_cp.wait()
    wr = wr_s[...].astype(f32).reshape(1, D)
    gate = jax.nn.sigmoid(jnp.sum(hn * wr, axis=-1, keepdims=True))
    set_columns(hn)

    g, u = zeros(F), zeros(F)
    for c, (lo, hi) in enumerate(up):
        g = gemv(g, wg_s, sem_g.at[c], lo, hi)
        u = gemv(u, wu_s, sem_u.at[c], lo, hi)
    g = fold(g)
    set_columns(g * jax.nn.sigmoid(g) * fold(u) * gate)

    resid = hres + hn
    top = lax.broadcasted_iota(jnp.int32, (8, 128), 0) == 0
    y = [jnp.where(top, resid[:, c:c + 128], 0.0) for c in range(0, D, 128)]
    for c, (lo, hi) in enumerate(down):
        y = gemv(y, wd_s, sem_d.at[c], lo, hi)
    o_ref[0] = fold(y).astype(o_ref.dtype)


@jax.jit
def pallas_sequential_preLN__sliding_block_cached__moe_arch_mod__decode_kernel(
    A_x: jax.Array,
    A_k_cache: jax.Array,
    A_v_cache: jax.Array,
    A_wq: jax.Array,
    A_wo: jax.Array,
    B_x: jax.Array,
    B_w_r: jax.Array,
    B_w_gate: jax.Array,
    B_w_up: jax.Array,
    B_w_down: jax.Array,
):
    del B_x
    _, H, Sk, Dh = A_k_cache.shape
    D = A_x.shape[-1]
    F = B_w_gate.shape[-1]
    W = min(4096, max(256, Sk // 4))
    kt = jnp.transpose(A_k_cache, (0, 1, 3, 2)).reshape(H, Dh, Sk)
    vt = jnp.transpose(A_v_cache, (0, 1, 3, 2)).reshape(H, Dh, Sk)
    wq, wo = (_tile_pairs(w, PROJ_STEPS) for w in (A_wq, A_wo))
    wg, wu, wd = (_tile_pairs(w, FFN_STEPS) for w in (B_w_gate, B_w_up, B_w_down))
    return pl.pallas_call(
        _kernel,
        out_shape=jax.ShapeDtypeStruct(A_x.shape, A_x.dtype),
        in_specs=[pl.BlockSpec(memory_space=pl.ANY)] * 9,
        scratch_shapes=[
            pltpu.VMEM(A_x.shape, A_x.dtype),
            pltpu.VMEM(B_w_r.shape, B_w_r.dtype),
            pltpu.VMEM((2, *wq.shape), wq.dtype),
            pltpu.VMEM((3, *wg.shape), wg.dtype),
            pltpu.VMEM((2, H, Dh, W), kt.dtype),
            pltpu.VMEM((4, 8, Dh), jnp.float32),
            pltpu.VMEM((H, 8, W), jnp.float32),
            pltpu.VMEM((H, 8, 128), jnp.float32),
            pltpu.VMEM((D // 128, 8, 128), jnp.float32),
            pltpu.VMEM((F, 128), jnp.float32),
            pltpu.SemaphoreType.DMA((H,)),
            pltpu.SemaphoreType.DMA((H,)),
            pltpu.SemaphoreType.DMA((4,)),
            pltpu.SemaphoreType.DMA((len(UP_CHUNKS),)),
            pltpu.SemaphoreType.DMA((len(UP_CHUNKS),)),
            pltpu.SemaphoreType.DMA((len(DOWN_CHUNKS),)),
        ],
        compiler_params=pltpu.CompilerParams(
            vmem_limit_bytes=126 * 2**20, disable_bounds_checks=True,
            disable_semaphore_checks=True),
    )(A_x, kt, vt, wq, wo, B_w_r, wg, wu, wd)
```

```python
import jax
import jax.numpy as jnp
from jax import lax
import jax.experimental.pallas as pl
import jax.experimental.pallas.tpu as pltpu

EPS = 1e-5
LOOK = 2
KV_ROWS, KV_COLS = 32, 512
AHEAD = 26
PROJ_STEPS = 15
PROJ_PAIR = (2, 3)
FFN_STEPS = 4
UP_CHUNKS = (40, 20)
DOWN_CHUNKS = (28, 16, 8, 4, 2, 1, 1)


def _layernorm(x):
    m = jnp.mean(x, axis=-1, keepdims=True)
    d = x - m
    v = jnp.mean(d * d, axis=-1, keepdims=True)
    return d / jnp.sqrt(v + EPS)


def _tile_pairs(w, steps):
    r, c = w.shape
    return w.reshape(r // 8, 8, c // 128, 128).transpose(0, 2, 1, 3).reshape(steps, -1, 16, 128)


def _ranges(sizes):
    out, lo = [], 0
    for n in sizes:
        out.append((lo, lo + n))
        lo += n
    return out


def _kernel(x_hbm, k_hbm, v_hbm, wq_hbm, wo_hbm, wr_hbm, wg_hbm, wu_hbm, wd_hbm, o_ref,
            x_s, wr_s, proj_s, ffn_s, kv_s, q_s, p_s, inv_s, acc_s, col_s,
            sem_k, sem_v, sem_w, sem_g, sem_u, sem_d):
    f32, bf16 = jnp.float32, jnp.bfloat16
    wq_s, wo_s = proj_s.at[0], proj_s.at[1]
    wg_s, wu_s, wd_s = ffn_s.at[0], ffn_s.at[1], ffn_s.at[2]
    k_s, v_s = kv_s.at[0], kv_s.at[1]
    _, H, Dh, W = kv_s.shape
    first = k_hbm.shape[-1] - W
    D = x_hbm.shape[-1]
    F = col_s.shape[0]
    n_d = D // 128

    def loop(lo, hi, body):
        lax.fori_loop(lo, hi, lambda i, _: body(i), None)

    def done(buf, sem):
        pltpu.make_async_copy(buf, buf, sem).wait()

    K, V = (k_hbm, k_s, sem_k), (v_hbm, v_s, sem_v)
    WQ, WO = (wq_hbm, wq_s, sem_w.at[0]), (wo_hbm, wo_s, sem_w.at[1])
    pairs = Dh // KV_ROWS // 2
    per_head = W // KV_COLS
    n_sweep = H * per_head

    def kv_start(arr, s, r, thread):
        src, dst, sem = arr
        h = s >> (per_head.bit_length() - 1)
        c = pl.multiple_of((s & (per_head - 1)) * KV_COLS, KV_COLS)
        r = (2 * r + thread) * KV_ROWS
        if not isinstance(r, int):
            r = pl.multiple_of(r, KV_ROWS)
        pltpu.make_async_copy(src.at[h, pl.ds(r, KV_ROWS), pl.ds(first + c, KV_COLS)],
                              dst.at[h, pl.ds(r, KV_ROWS), pl.ds(c, KV_COLS)],
                              sem.at[h]).start(priority=thread)

    proj_pairs = PROJ_STEPS // sum(PROJ_PAIR)

    def proj_start(arr, u, r, thread):
        src, dst, sem = arr
        rows = pl.ds(r * sum(PROJ_PAIR) + thread * PROJ_PAIR[0], PROJ_PAIR[thread])
        idx = (rows, pl.ds(2 * u, 2))
        pltpu.make_async_copy(src.at[idx], dst.at[idx], sem).start(priority=thread)

    def proj_sweep(arr0, u0, arr1, u1):
        for r in range(proj_pairs):
            proj_start(arr0, u0, r, 0)
            proj_start(arr1, u1, r, 1)

    n_ffn = wd_s.shape[1] // 2
    up, down = _ranges(UP_CHUNKS), _ranges(DOWN_CHUNKS)
    FFN = {"g": (wg_hbm, wg_s, sem_g, up), "u": (wu_hbm, wu_s, sem_u, up),
           "d": (wd_hbm, wd_s, sem_d, down)}

    def ffn_start(name, u, thread):
        src, dst, sems, chunks = FFN[name]
        c = next(i for i, (lo, hi) in enumerate(chunks) if lo <= u < hi)
        idx = (slice(None), pl.ds(2 * u, 2))
        pltpu.make_async_copy(src.at[idx], dst.at[idx], sems.at[c]).start(priority=thread)

    order = [(a, u) for u in range(n_ffn) for a in "gu"] + [("d", u) for u in range(n_ffn)]
    paired = len(order) - AHEAD
    ffn0 = order[0:paired:2]
    ffn1 = order[1:paired:2] + order[paired:]
    assert ffn1[:AHEAD] == [("u", u) for u in range(AHEAD)] and up[0][1] >= AHEAD

    def ffn_part(part):
        n = pl.cdiv(len(ffn0), 3)
        for i in range(part * n, min((part + 1) * n, len(ffn0))):
            ffn_start(*ffn0[i], 0)
            ffn_start(*ffn1[AHEAD + i], 1)

    def k1(s, r):
        kv_start(K, s, r, 1)

    def v1(s, r):
        kv_start(V, s - n_sweep, r, 1)

    def u1(s, r):
        idx = (slice(None), pl.ds(2 * ((s - 2 * n_sweep) * pairs + r), 2))
        pltpu.make_async_copy(wu_hbm.at[idx], wu_s.at[idx], sem_u.at[0]).start(priority=1)

    whole, part = divmod(AHEAD, pairs)

    def stage(arr0, before, this, following):
        def body(s):
            for r in range(pairs):
                kv_start(arr0, s - before, r, 0)
                carry, r1 = divmod(r + part, pairs)
                (following if carry else this)(s + whole + carry, r1)
        return body

    turn = n_sweep - whole
    stages = ((0, turn - 1, stage(K, 0, k1, k1)),
              (turn - 1, turn, stage(K, 0, k1, v1)),
              (turn, n_sweep, stage(K, 0, v1, v1)),
              (n_sweep, n_sweep + turn - 1, stage(V, n_sweep, v1, v1)),
              (n_sweep + turn - 1, n_sweep + turn, stage(V, n_sweep, v1, u1)),
              (n_sweep + turn, 2 * n_sweep, stage(V, n_sweep, u1, u1)))

    def head_start(j, which):
        for lo, hi, body in which:
            loop(jnp.clip(j * per_head, lo, hi), jnp.clip((j + 1) * per_head, lo, hi), body)

    x_cp = pltpu.make_async_copy(x_hbm, x_s, sem_w.at[2])
    wr_cp = pltpu.make_async_copy(wr_hbm, wr_s, sem_w.at[3])

    n_u = wq_s.shape[1] // 2
    lead = pl.cdiv(AHEAD, proj_pairs)
    both = n_u - lead
    for u in range(lead):
        for r in range(proj_pairs):
            proj_start(WQ, u, r, 1)
    loop(0, both, lambda u: proj_sweep(WQ, u, WQ, u + lead))
    x_cp.start()
    wr_cp.start()
    loop(both, n_u, lambda u: proj_sweep(WQ, u, WO, u - both))
    loop(0, both, lambda u: proj_sweep(WO, u, WO, u + lead))

    def wo_to_k(u):
        for r in range(proj_pairs):
            j = (u - both) * proj_pairs + r
            proj_start(WO, u, r, 0)
            pl.when(j < AHEAD)(lambda j=j: k1(j // pairs, j % pairs))

    loop(both, n_u, wo_to_k)
    loop(0, LOOK * per_head, stages[0][2])

    def set_columns(row):
        for b in range(0, row.shape[1], 128):
            col_s[b:b + 128, :] = jnp.broadcast_to(row[:, b:b + 128], (128, 128)).T

    def zeros(n):
        return [jnp.zeros((8, 128), f32)] * (n // 128)

    def fold(acc):
        return jnp.concatenate([jnp.sum(a, axis=0, keepdims=True) for a in acc], axis=1)

    def proj_block(ref, b):
        n = ref.shape[1]
        assert n & (n - 1) == 0
        return ref[b >> (n.bit_length() - 1), b & (n - 1)].astype(f32)

    x_cp.wait()
    x = x_s[0].astype(f32)
    set_columns(_layernorm(x))
    done(wq_s, sem_w.at[0])

    def k_step(h):
        head_start(h + LOOK, stages[:4])

        @pl.when(h % 4 == 0)
        def _():
            acc = list(zeros(4 * Dh))
            per_row = H * Dh // 256
            for g in range(D // 8):
                xc = col_s[8 * g:8 * g + 8, :]
                for i in range(len(acc) // 2):
                    ww = proj_block(wq_s, per_row * g + i + (h // 4) * (len(acc) // 2))
                    acc[2 * i] = acc[2 * i] + ww[:8] * xc
                    acc[2 * i + 1] = acc[2 * i + 1] + ww[8:] * xc
            q4 = jnp.broadcast_to(fold(acc), (8, 4 * Dh))
            for i in range(4):
                q_s[i] = q4[:, i * Dh:(i + 1) * Dh]

        done(k_s.at[h], sem_k.at[h])
        s = jnp.dot(q_s[h % 4].astype(bf16), k_s[h], preferred_element_type=f32) * Dh ** -0.5
        e = jnp.exp(s - jnp.max(s, axis=-1, keepdims=True))
        p_s[h] = e
        inv_s[h] = jnp.broadcast_to(1.0 / jnp.sum(e, axis=-1, keepdims=True), (8, 128))

    loop(0, H, k_step)

    acc_s[...] = jnp.zeros_like(acc_s)
    done(wo_s, sem_w.at[1])

    def v_step(h):
        head_start(H + h + LOOK, stages[3:])
        pl.when(h + LOOK == H)(lambda: ffn_part(0))
        pl.when(h + LOOK == H + 1)(lambda: ffn_part(1))

        done(v_s.at[h], sem_v.at[h])
        inv = inv_s[h][:, :1]
        acc = [acc_s[c] for c in range(n_d)]
        for r in range(Dh // 16):
            a0 = jnp.zeros((8, 128), f32)
            a1 = jnp.zeros((8, 128), f32)
            for c in range(0, W, 128):
                pp = p_s[h, :, c:c + 128]
                vv = v_s[h, r * 16:(r + 1) * 16, c:c + 128].astype(f32)
                a0 = a0 + vv[:8] * pp
                a1 = a1 + vv[8:] * pp
            o = [jnp.sum(a, axis=-1, keepdims=True) * inv for a in (a0, a1)]
            for b in range(n_d):
                ww = proj_block(wo_s, (h * (Dh // 16) + r) * n_d + b)
                for t in range(2):
                    g, c = divmod(2 * b + t, n_d)
                    acc[c] = acc[c] + ww[8 * t:8 * t + 8] * o[g]
        for c in range(n_d):
            acc_s[c] = acc[c]

    loop(0, H, v_step)
    ffn_part(2)

    def gemv(acc, w_s, sem, lo, hi):
        done(w_s.at[:, 2 * lo:2 * hi], sem)
        acc = list(acc)
        for b in range(2 * lo, 2 * hi):
            for s in range(w_s.shape[0]):
                ww = w_s[s, b].astype(f32)
                for t in range(2):
                    g, c = divmod(2 * (s * w_s.shape[1] + b) + t, len(acc))
                    acc[c] = acc[c] + ww[8 * t:8 * t + 8] * col_s[8 * g:8 * g + 8, :]
        return acc

    hres = x + fold([acc_s[c] for c in range(n_d)])
    hn = _layernorm(hres)
    wr_cp.wait()
    wr = wr_s[...].astype(f32).reshape(1, D)
    gate = jax.nn.sigmoid(jnp.sum(hn * wr, axis=-1, keepdims=True))
    set_columns(hn)

    g, u = zeros(F), zeros(F)
    for c, (lo, hi) in enumerate(up):
        g = gemv(g, wg_s, sem_g.at[c], lo, hi)
        u = gemv(u, wu_s, sem_u.at[c], lo, hi)
    g = fold(g)
    set_columns(g * jax.nn.sigmoid(g) * fold(u) * gate)

    resid = hres + hn
    top = lax.broadcasted_iota(jnp.int32, (8, 128), 0) == 0
    y = [jnp.where(top, resid[:, c:c + 128], 0.0) for c in range(0, D, 128)]
    for c, (lo, hi) in enumerate(down):
        y = gemv(y, wd_s, sem_d.at[c], lo, hi)
    o_ref[0] = fold(y).astype(o_ref.dtype)


@jax.jit
def pallas_sequential_preLN__sliding_block_cached__moe_arch_mod__decode_kernel(
    A_x: jax.Array,
    A_k_cache: jax.Array,
    A_v_cache: jax.Array,
    A_wq: jax.Array,
    A_wo: jax.Array,
    B_x: jax.Array,
    B_w_r: jax.Array,
    B_w_gate: jax.Array,
    B_w_up: jax.Array,
    B_w_down: jax.Array,
):
    del B_x
    _, H, Sk, Dh = A_k_cache.shape
    D = A_x.shape[-1]
    F = B_w_gate.shape[-1]
    W = min(4096, max(256, Sk // 4))
    kt = jnp.transpose(A_k_cache, (0, 1, 3, 2)).reshape(H, Dh, Sk)
    vt = jnp.transpose(A_v_cache, (0, 1, 3, 2)).reshape(H, Dh, Sk)
    wq, wo = (_tile_pairs(w, PROJ_STEPS) for w in (A_wq, A_wo))
    wg, wu, wd = (_tile_pairs(w, FFN_STEPS) for w in (B_w_gate, B_w_up, B_w_down))
    return pl.pallas_call(
        _kernel,
        out_shape=jax.ShapeDtypeStruct(A_x.shape, A_x.dtype),
        in_specs=[pl.BlockSpec(memory_space=pl.ANY)] * 9,
        scratch_shapes=[
            pltpu.VMEM(A_x.shape, A_x.dtype),
            pltpu.VMEM(B_w_r.shape, B_w_r.dtype),
            pltpu.VMEM((2, *wq.shape), wq.dtype),
            pltpu.VMEM((3, *wg.shape), wg.dtype),
            pltpu.VMEM((2, H, Dh, W), kt.dtype),
            pltpu.VMEM((4, 8, Dh), jnp.float32),
            pltpu.VMEM((H, 8, W), jnp.float32),
            pltpu.VMEM((H, 8, 128), jnp.float32),
            pltpu.VMEM((D // 128, 8, 128), jnp.float32),
            pltpu.VMEM((F, 128), jnp.float32),
            pltpu.SemaphoreType.DMA((H,)),
            pltpu.SemaphoreType.DMA((H,)),
            pltpu.SemaphoreType.DMA((4,)),
            pltpu.SemaphoreType.DMA((len(UP_CHUNKS),)),
            pltpu.SemaphoreType.DMA((len(UP_CHUNKS),)),
            pltpu.SemaphoreType.DMA((len(DOWN_CHUNKS),)),
        ],
        compiler_params=pltpu.CompilerParams(
            vmem_limit_bytes=126 * 2**20, disable_bounds_checks=True,
            disable_semaphore_checks=True),
    )(A_x, kt, vt, wq, wo, B_w_r, wg, wu, wd)
```

```python
import jax
import jax.numpy as jnp
from jax import lax
import jax.experimental.pallas as pl
import jax.experimental.pallas.tpu as pltpu

EPS = 1e-5
LOOK = 2
KV_ROWS, KV_COLS = 32, 512
AHEAD = 26
PROJ_STEPS = 15
PROJ_PAIR = (2, 3)
FFN_STEPS = 4
DOWN_CHUNKS = (40, 12, 5, 2, 1)


def _layernorm(x):
    m = jnp.mean(x, axis=-1, keepdims=True)
    d = x - m
    v = jnp.mean(d * d, axis=-1, keepdims=True)
    return d / jnp.sqrt(v + EPS)


def _tile_pairs(w, steps):
    r, c = w.shape
    return w.reshape(r // 8, 8, c // 128, 128).transpose(0, 2, 1, 3).reshape(steps, -1, 16, 128)


def _ranges(sizes):
    out, lo = [], 0
    for n in sizes:
        out.append((lo, lo + n))
        lo += n
    return out


def _kernel(x_hbm, k_hbm, v_hbm, wq_hbm, wo_hbm, wr_hbm, wg_hbm, wu_hbm, wd_hbm, o_ref,
            x_s, wr_s, proj_s, ffn_s, kv_s, q_s, p_s, inv_s, acc_s, col_s,
            sem_k, sem_v, sem_w, sem_d):
    f32, bf16 = jnp.float32, jnp.bfloat16
    wq_s, wo_s = proj_s.at[0], proj_s.at[1]
    wg_s, wu_s, wd_s = ffn_s.at[0], ffn_s.at[1], ffn_s.at[2]
    k_s, v_s = kv_s.at[0], kv_s.at[1]
    _, H, Dh, W = kv_s.shape
    first = k_hbm.shape[-1] - W
    D = x_hbm.shape[-1]
    F = col_s.shape[0]
    n_d = D // 128

    def loop(lo, hi, body):
        lax.fori_loop(lo, hi, lambda i, _: body(i), None)

    def done(buf, sem):
        pltpu.make_async_copy(buf, buf, sem).wait()

    K, V = (k_hbm, k_s, sem_k), (v_hbm, v_s, sem_v)
    WQ, WO = (wq_hbm, wq_s, sem_w.at[0]), (wo_hbm, wo_s, sem_w.at[1])
    pairs = Dh // KV_ROWS // 2
    per_head = W // KV_COLS
    n_sweep = H * per_head

    def kv_start(arr, s, r, thread):
        src, dst, sem = arr
        h = s >> (per_head.bit_length() - 1)
        c = pl.multiple_of((s & (per_head - 1)) * KV_COLS, KV_COLS)
        r = (2 * r + thread) * KV_ROWS
        if not isinstance(r, int):
            r = pl.multiple_of(r, KV_ROWS)
        pltpu.make_async_copy(src.at[h, pl.ds(r, KV_ROWS), pl.ds(first + c, KV_COLS)],
                              dst.at[h, pl.ds(r, KV_ROWS), pl.ds(c, KV_COLS)],
                              sem.at[h]).start(priority=thread)

    proj_pairs = PROJ_STEPS // sum(PROJ_PAIR)

    def proj_start(arr, u, r, thread):
        src, dst, sem = arr
        rows = pl.ds(r * sum(PROJ_PAIR) + thread * PROJ_PAIR[0], PROJ_PAIR[thread])
        idx = (rows, pl.ds(2 * u, 2))
        pltpu.make_async_copy(src.at[idx], dst.at[idx], sem).start(priority=thread)

    def proj_sweep(arr0, u0, arr1, u1):
        for r in range(proj_pairs):
            proj_start(arr0, u0, r, 0)
            proj_start(arr1, u1, r, 1)

    n_ffn = wd_s.shape[1] // 2
    down = _ranges(DOWN_CHUNKS)
    WG, WU = (wg_hbm, wg_s, sem_w.at[2]), (wu_hbm, wu_s, sem_w.at[3])

    def ffn_start(arr, u, thread):
        src, dst, sem = arr
        idx = (slice(None), pl.ds(2 * u, 2))
        pltpu.make_async_copy(src.at[idx], dst.at[idx], sem).start(priority=thread)

    order = [(arr, u) for u in range(n_ffn) for arr in (WG, WU)]
    order += [((wd_hbm, wd_s, sem_d.at[c]), u)
              for c, (lo, hi) in enumerate(down) for u in range(lo, hi)]
    paired = len(order) - AHEAD
    ffn0 = order[0:paired:2]
    ffn1 = order[1:paired:2] + order[paired:]

    def ffn_part(part):
        n = pl.cdiv(len(ffn0), 3)
        for i in range(part * n, min((part + 1) * n, len(ffn0))):
            ffn_start(*ffn0[i], 0)
            ffn_start(*ffn1[AHEAD + i], 1)

    def k1(s, r):
        kv_start(K, s, r, 1)

    def v1(s, r):
        kv_start(V, s - n_sweep, r, 1)

    def u1(s, r):
        ffn_start(WU, (s - 2 * n_sweep) * pairs + r, 1)

    whole, part = divmod(AHEAD, pairs)

    def stage(arr0, before, this, following):
        def body(s):
            for r in range(pairs):
                kv_start(arr0, s - before, r, 0)
                carry, r1 = divmod(r + part, pairs)
                (following if carry else this)(s + whole + carry, r1)
        return body

    turn = n_sweep - whole
    stages = ((0, turn - 1, stage(K, 0, k1, k1)),
              (turn - 1, turn, stage(K, 0, k1, v1)),
              (turn, n_sweep, stage(K, 0, v1, v1)),
              (n_sweep, n_sweep + turn - 1, stage(V, n_sweep, v1, v1)),
              (n_sweep + turn - 1, n_sweep + turn, stage(V, n_sweep, v1, u1)),
              (n_sweep + turn, 2 * n_sweep, stage(V, n_sweep, u1, u1)))

    def head_start(j, which):
        for lo, hi, body in which:
            loop(jnp.clip(j * per_head, lo, hi), jnp.clip((j + 1) * per_head, lo, hi), body)

    x_cp = pltpu.make_async_copy(x_hbm, x_s, sem_w.at[4])
    wr_cp = pltpu.make_async_copy(wr_hbm, wr_s, sem_w.at[5])

    n_u = wq_s.shape[1] // 2
    lead = pl.cdiv(AHEAD, proj_pairs)
    both = n_u - lead
    for u in range(lead):
        for r in range(proj_pairs):
            proj_start(WQ, u, r, 1)
    loop(0, both, lambda u: proj_sweep(WQ, u, WQ, u + lead))
    x_cp.start()
    wr_cp.start()
    loop(both, n_u, lambda u: proj_sweep(WQ, u, WO, u - both))
    loop(0, both, lambda u: proj_sweep(WO, u, WO, u + lead))

    def wo_to_k(u):
        for r in range(proj_pairs):
            j = (u - both) * proj_pairs + r
            proj_start(WO, u, r, 0)
            pl.when(j < AHEAD)(lambda j=j: k1(j // pairs, j % pairs))

    loop(both, n_u, wo_to_k)
    loop(0, LOOK * per_head, stages[0][2])

    def set_columns(row):
        for b in range(0, row.shape[1], 128):
            col_s[b:b + 128, :] = jnp.broadcast_to(row[:, b:b + 128], (128, 128)).T

    def zeros(n):
        return [jnp.zeros((8, 128), f32)] * (n // 128)

    def fold(acc):
        return jnp.concatenate([jnp.sum(a, axis=0, keepdims=True) for a in acc], axis=1)

    def proj_block(ref, b):
        n = ref.shape[1]
        assert n & (n - 1) == 0
        return ref[b >> (n.bit_length() - 1), b & (n - 1)].astype(f32)

    x_cp.wait()
    x = x_s[0].astype(f32)
    set_columns(_layernorm(x))
    done(wq_s, sem_w.at[0])

    def k_step(h):
        head_start(h + LOOK, stages[:4])

        @pl.when(h % 4 == 0)
        def _():
            acc = list(zeros(4 * Dh))
            per_row = H * Dh // 256
            for g in range(D // 8):
                xc = col_s[8 * g:8 * g + 8, :]
                for i in range(len(acc) // 2):
                    ww = proj_block(wq_s, per_row * g + i + (h // 4) * (len(acc) // 2))
                    acc[2 * i] = acc[2 * i] + ww[:8] * xc
                    acc[2 * i + 1] = acc[2 * i + 1] + ww[8:] * xc
            q4 = jnp.broadcast_to(fold(acc), (8, 4 * Dh))
            for i in range(4):
                q_s[i] = q4[:, i * Dh:(i + 1) * Dh]

        done(k_s.at[h], sem_k.at[h])
        s = jnp.dot(q_s[h % 4].astype(bf16), k_s[h], preferred_element_type=f32) * Dh ** -0.5
        e = jnp.exp(s - jnp.max(s, axis=-1, keepdims=True))
        p_s[h] = e
        inv_s[h] = jnp.broadcast_to(1.0 / jnp.sum(e, axis=-1, keepdims=True), (8, 128))

    loop(0, H, k_step)

    acc_s[...] = jnp.zeros_like(acc_s)
    done(wo_s, sem_w.at[1])

    def v_step(h):
        head_start(H + h + LOOK, stages[3:])
        pl.when(h + LOOK == H)(lambda: ffn_part(0))
        pl.when(h + LOOK == H + 1)(lambda: ffn_part(1))

        done(v_s.at[h], sem_v.at[h])
        inv = inv_s[h][:, :1]
        acc = [acc_s[c] for c in range(n_d)]
        for r in range(Dh // 16):
            a0 = jnp.zeros((8, 128), f32)
            a1 = jnp.zeros((8, 128), f32)
            for c in range(0, W, 128):
                pp = p_s[h, :, c:c + 128]
                vv = v_s[h, r * 16:(r + 1) * 16, c:c + 128].astype(f32)
                a0 = a0 + vv[:8] * pp
                a1 = a1 + vv[8:] * pp
            o = [jnp.sum(a, axis=-1, keepdims=True) * inv for a in (a0, a1)]
            for b in range(n_d):
                ww = proj_block(wo_s, (h * (Dh // 16) + r) * n_d + b)
                for t in range(2):
                    g, c = divmod(2 * b + t, n_d)
                    acc[c] = acc[c] + ww[8 * t:8 * t + 8] * o[g]
        for c in range(n_d):
            acc_s[c] = acc[c]

    loop(0, H, v_step)
    ffn_part(2)

    def gemv(acc, w_s, sem, lo, hi):
        done(w_s.at[:, 2 * lo:2 * hi], sem)
        acc = list(acc)
        for b in range(2 * lo, 2 * hi):
            for s in range(w_s.shape[0]):
                ww = w_s[s, b].astype(f32)
                for t in range(2):
                    g, c = divmod(2 * (s * w_s.shape[1] + b) + t, len(acc))
                    acc[c] = acc[c] + ww[8 * t:8 * t + 8] * col_s[8 * g:8 * g + 8, :]
        return acc

    hres = x + fold([acc_s[c] for c in range(n_d)])
    hn = _layernorm(hres)
    wr_cp.wait()
    wr = wr_s[...].astype(f32).reshape(1, D)
    gate = jax.nn.sigmoid(jnp.sum(hn * wr, axis=-1, keepdims=True))
    set_columns(hn)

    g = fold(gemv(zeros(F), wg_s, WG[2], 0, n_ffn))
    u = fold(gemv(zeros(F), wu_s, WU[2], 0, n_ffn))
    set_columns(g * jax.nn.sigmoid(g) * u * gate)

    resid = hres + hn
    top = lax.broadcasted_iota(jnp.int32, (8, 128), 0) == 0
    y = [jnp.where(top, resid[:, c:c + 128], 0.0) for c in range(0, D, 128)]
    for c, (lo, hi) in enumerate(down):
        y = gemv(y, wd_s, sem_d.at[c], lo, hi)
    o_ref[0] = fold(y).astype(o_ref.dtype)


@jax.jit
def pallas_sequential_preLN__sliding_block_cached__moe_arch_mod__decode_kernel(
    A_x: jax.Array,
    A_k_cache: jax.Array,
    A_v_cache: jax.Array,
    A_wq: jax.Array,
    A_wo: jax.Array,
    B_x: jax.Array,
    B_w_r: jax.Array,
    B_w_gate: jax.Array,
    B_w_up: jax.Array,
    B_w_down: jax.Array,
):
    del B_x
    _, H, Sk, Dh = A_k_cache.shape
    D = A_x.shape[-1]
    F = B_w_gate.shape[-1]
    W = min(4096, max(256, Sk // 4))
    kt = jnp.transpose(A_k_cache, (0, 1, 3, 2)).reshape(H, Dh, Sk)
    vt = jnp.transpose(A_v_cache, (0, 1, 3, 2)).reshape(H, Dh, Sk)
    wq, wo = (_tile_pairs(w, PROJ_STEPS) for w in (A_wq, A_wo))
    wg, wu, wd = (_tile_pairs(w, FFN_STEPS) for w in (B_w_gate, B_w_up, B_w_down))
    return pl.pallas_call(
        _kernel,
        out_shape=jax.ShapeDtypeStruct(A_x.shape, A_x.dtype),
        in_specs=[pl.BlockSpec(memory_space=pl.ANY)] * 9,
        scratch_shapes=[
            pltpu.VMEM(A_x.shape, A_x.dtype),
            pltpu.VMEM(B_w_r.shape, B_w_r.dtype),
            pltpu.VMEM((2, *wq.shape), wq.dtype),
            pltpu.VMEM((3, *wg.shape), wg.dtype),
            pltpu.VMEM((2, H, Dh, W), kt.dtype),
            pltpu.VMEM((4, 8, Dh), jnp.float32),
            pltpu.VMEM((H, 8, W), jnp.float32),
            pltpu.VMEM((H, 8, 128), jnp.float32),
            pltpu.VMEM((D // 128, 8, 128), jnp.float32),
            pltpu.VMEM((F, 128), jnp.float32),
            pltpu.SemaphoreType.DMA((H,)),
            pltpu.SemaphoreType.DMA((H,)),
            pltpu.SemaphoreType.DMA((6,)),
            pltpu.SemaphoreType.DMA((len(DOWN_CHUNKS),)),
        ],
        compiler_params=pltpu.CompilerParams(
            vmem_limit_bytes=126 * 2**20, disable_semaphore_checks=True),
    )(A_x, kt, vt, wq, wo, B_w_r, wg, wu, wd)
```
